```python
import jax
import jax.numpy as jnp

def _softmax(x, axis=-1):
    return jax.nn.softmax(x, axis=axis)
def _gelu(x):
    return jax.nn.gelu(x, approximate=True)
def _silu(x):
    return jax.nn.silu(x)
def _sigmoid(x):
    return jax.nn.sigmoid(x)
def _layernorm(x, axis=-1, eps=1e-5):
    m = jnp.mean(x, axis=axis, keepdims=True)
    v = jnp.var(x, axis=axis, keepdims=True)
    return (x - m) / jnp.sqrt(v + eps)
def _scatter_add(tgt, idx, src, axis=0):
    return tgt.at[idx].add(src)
def _segment_sum(src, seg, n):
    return jax.ops.segment_sum(src, seg, n)
class _Rng:
    def __init__(self, key):
        self._k = key
    def _next(self):
        self._k, sub = jax.random.split(self._k)
        return sub
    def normal(self, shape):
        return jax.random.normal(self._next(), shape, dtype=jnp.bfloat16)
    def randint(self, lo, hi, shape):
        return jax.random.randint(self._next(), shape, lo, hi, dtype=jnp.int32)
    def uniform(self, shape, lo=0.0, hi=1.0):
        return jax.random.uniform(self._next(), shape, jnp.bfloat16, lo, hi)
    def permutation(self, n):
        return jax.random.permutation(self._next(), n)


kernel_name = 'sequential_preLN__sliding_block_cached__moe_arch_mod__decode'

def setup_inputs():
    _rng = _Rng(jax.random.key(int.from_bytes(__import__("os").urandom(4), "little")))
    _w = (lambda a: (lambda t: t.astype(jnp.bfloat16) if jnp.issubdtype(t.dtype, jnp.floating) else t)(jnp.asarray(a)))
    def _A_setup():
        B, Sq, D = 1, 1, 640
        Hq, Hkv, Sk, Dh = 32, 32, 32768, 192
        assert Hq % Hkv == 0, (Hq, Hkv)
        return {
            "x": _w((lambda *s: _rng.normal(s) * 0.05)(B, Sq, D)),
            "k_cache": _w((lambda *s: _rng.normal(s) * 0.05)(B, Hkv, Sk, Dh)),
            "v_cache": _w((lambda *s: _rng.normal(s) * 0.05)(B, Hkv, Sk, Dh)),
            "wq": _w((lambda *s: _rng.normal(s) * 0.05)(D, Hq * Dh) * (D ** -0.5)),
            "wo": _w((lambda *s: _rng.normal(s) * 0.05)(Hq * Dh, D) * ((Hq * Dh) ** -0.5)),
        }
    _A_in = _A_setup()

    def _B_setup():
        B, S, D, F, C = 1, 1, 640, 1536, 1
        return {
            "x": _w((lambda *s: _rng.normal(s) * 0.05)(B, S, D)),
            "w_r": _w((lambda *s: _rng.normal(s) * 0.05)(D)),
            "w_gate": _w((lambda *s: _rng.normal(s) * 0.05)(D, F)),
            "w_up": _w((lambda *s: _rng.normal(s) * 0.05)(D, F)),
            "w_down": _w((lambda *s: _rng.normal(s) * 0.05)(F, D)),
        }
    _B_in = _B_setup()

    return {
        "A_x": _A_in["x"],
        "A_k_cache": _A_in["k_cache"],
        "A_v_cache": _A_in["v_cache"],
        "A_wq": _A_in["wq"],
        "A_wo": _A_in["wo"],
        "B_x": _B_in["x"],
        "B_w_r": _B_in["w_r"],
        "B_w_gate": _B_in["w_gate"],
        "B_w_up": _B_in["w_up"],
        "B_w_down": _B_in["w_down"],
    }

def reference(A_x, A_k_cache, A_v_cache, A_wq, A_wo, B_x, B_w_r, B_w_gate, B_w_up, B_w_down):
    def _A_ref(x, k_cache, v_cache, wq, wo):
        B, Sq, D = x.shape
        Hq, Dh = 32, 192
        Hkv, Sk = k_cache.shape[1], k_cache.shape[2]
        W = min(4096, max(256, Sk // 4))
        rep = Hq // Hkv
        q = (lambda x, *d: x.transpose(*d))((x @ wq).reshape(B, Sq, Hq, Dh), 0, 2, 1, 3)
        k = jnp.repeat(k_cache[:, :, Sk - W:, :], rep, axis=1)
        v = jnp.repeat(v_cache[:, :, Sk - W:, :], rep, axis=1)
        scores = jnp.einsum("bhqd,bhkd->bhqk", q, k) * (Dh ** -0.5)
        p = _softmax(scores, axis=-1)
        o = jnp.einsum("bhqk,bhkd->bhqd", p, v)
        return (lambda x, *d: x.transpose(*d))(o, 0, 2, 1, 3).reshape(B, Sq, Hq * Dh) @ wo

    def _B_ref(x, w_r, w_gate, w_up, w_down):
        B, S, D = x.shape
        C = 1
        r = x @ w_r
        idx = jnp.argsort(-r, axis=-1)[:, :C]
        idx_e = jnp.repeat(idx.reshape(B, C, 1), D, axis=2)
        x_sel = jnp.take_along_axis(x, idx_e, axis=1)
        g = _silu(x_sel @ w_gate)
        u = x_sel @ w_up
        y = (g * u) @ w_down
        r_sel = _sigmoid(jnp.take_along_axis(r, idx, axis=1))
        y = y * r_sel.reshape(B, C, 1)
        b_off = (jnp.arange(B) * S).reshape(B, 1)
        flat_idx = (idx + b_off).reshape(B * C)
        zero = (x * 0.0).reshape(B * S, D)
        upd = _scatter_add(zero, flat_idx, y.reshape(B * C, D), axis=0)
        return x + upd.reshape(B, S, D)

    x = A_x
    h = x + _A_ref(_layernorm(x, axis=-1), A_k_cache, A_v_cache, A_wq, A_wo)
    h2 = h + _B_ref(_layernorm(h, axis=-1), B_w_r, B_w_gate, B_w_up, B_w_down)
    return h2
```

```python
import functools

import jax
import jax.numpy as jnp
from jax import lax
import jax.experimental.pallas as pl
import jax.experimental.pallas.tpu as pltpu

D = 640
H = 32
DH = 192
SK = 32768
W = 4096
F = 1536
EPS = 1e-5
SCALE = 0.072265625

CH = 128
NC = W // CH
R = 4
DEPTH = NC
LEAD = 8
LO, HI = 1, 0

WQ_ROWS = 8
NQ = D // WQ_ROWS
WO_ROWS = 48
NO = H * DH // WO_ROWS // 2
NA = NQ + NO
G_ROWS = 16
NG = D // G_ROWS
DN_ROWS = 32
ND = F // DN_ROWS // 2
DN_BLK = 128
NT = NG + ND


def _layernorm(v):
    m = jnp.mean(v, axis=-1, keepdims=True)
    c = v - m
    var = jnp.mean(c * c, axis=-1, keepdims=True)
    return c / jnp.sqrt(var + EPS)


def _row8(v):
    return jnp.broadcast_to(v, (8, v.shape[1])).astype(jnp.bfloat16)


def _kernel(x_hbm, k_hbm, v_hbm, wq_hbm, wo_hbm, wr_hbm, wg_hbm, wu_hbm, wd_hbm,
            o_ref,
            kbuf, vbuf, wq_buf, wo_buf, wg_buf, wu_buf, wd_buf, x_buf, wr_buf,
            q_buf, s_buf, acc_buf,
            sem_k, sem_v, sem_w, sem_d):
    cp = pltpu.make_async_copy

    def rows(start, n, align):
        if isinstance(start, int):
            return pl.ds(start, n)
        return pl.ds(pl.multiple_of(start, align), n)

    def wq_chunk(i, half):
        r = rows(i * WQ_ROWS, WQ_ROWS, WQ_ROWS)
        c = pl.ds(half * (H * DH // 2), H * DH // 2)
        return cp(wq_hbm.at[r, c], wq_buf.at[r, c], sem_w.at[half])

    def wo_chunk(i, half):
        r = rows((i * 2 + half) * WO_ROWS, WO_ROWS, WO_ROWS)
        return cp(wo_hbm.at[r, :], wo_buf.at[r, :], sem_w.at[2 + half])

    def kv_chunk(src, dst, sem, h, c):
        slot = h % R
        return cp(src.at[h, :, pl.ds(SK - W + c * CH, CH)],
                  dst.at[slot, :, pl.ds(c * CH, CH)], sem.at[slot])

    def k_chunk(h, c):
        return kv_chunk(k_hbm, kbuf, sem_k, h, c)

    def v_chunk(h, c):
        return kv_chunk(v_hbm, vbuf, sem_v, h, c)

    def tail_chunk(i, half):
        if i < NG:
            r = pl.ds(i * G_ROWS, G_ROWS)
            if half == 0:
                return cp(wg_hbm.at[r, :], wg_buf.at[r, :], sem_w.at[4])
            return cp(wu_hbm.at[r, :], wu_buf.at[r, :], sem_w.at[5])
        j = i - NG
        r = pl.ds((2 * j + half) * DN_ROWS, DN_ROWS)
        return cp(wd_hbm.at[r, :], wd_buf.at[r, :],
                  sem_d.at[half * (F // DN_BLK) + (2 * j * DN_ROWS) // DN_BLK])

    def wait_all(buf, sem):
        cp(buf, buf, sem).wait()

    for i in range(LEAD):
        wq_chunk(i, 1).start(priority=HI)
        wq_chunk(i, 0).start(priority=LO)
    x_copy = cp(x_hbm, x_buf, sem_w.at[6])
    wr_copy = cp(wr_hbm, wr_buf, sem_w.at[7])
    x_copy.start(priority=HI)
    wr_copy.start(priority=HI)
    for i in range(LEAD, DEPTH):
        wq_chunk(i, 0).start(priority=LO)

    def a1_body(t, carry):
        wq_chunk(t, 0).wait()
        wq_chunk(t + LEAD, 1).start(priority=HI)
        wq_chunk(t + DEPTH, 0).start(priority=LO)
        return carry
    lax.fori_loop(0, NQ - DEPTH, a1_body, 0)

    def a2_body(t, carry):
        wq_chunk(t, 0).wait()
        wq_chunk(t + LEAD, 1).start(priority=HI)
        wo_chunk(t + DEPTH - NQ, 0).start(priority=LO)
        return carry
    lax.fori_loop(NQ - DEPTH, NQ - LEAD, a2_body, 0)

    def a3_body(t, carry):
        wq_chunk(t, 0).wait()
        wo_chunk(t + LEAD - NQ, 1).start(priority=HI)
        wo_chunk(t + DEPTH - NQ, 0).start(priority=LO)
        return carry
    lax.fori_loop(NQ - LEAD, NQ, a3_body, 0)

    x_copy.wait()
    wr_copy.wait()
    x = x_buf[...].astype(jnp.float32)
    xn8 = _row8(_layernorm(x))
    half_q = wq_buf.at[:, pl.ds(H * DH // 2, H * DH // 2)]
    cp(half_q, half_q, sem_w.at[1]).wait()

    def q_piece(j):
        col = pl.multiple_of(j * (2 * DH), 128)
        q2 = jnp.dot(xn8, wq_buf[:, pl.ds(col, 2 * DH)],
                     preferred_element_type=jnp.float32)
        q_buf[pl.ds(2 * j, 1), :] = q2[0:1, 0:DH]
        q_buf[pl.ds(2 * j + 1, 1), :] = q2[0:1, DH:2 * DH]

    def wo_step(t):
        wo_chunk(t, 0).wait()

        @pl.when(t + LEAD < NO)
        def _():
            wo_chunk(t + LEAD, 1).start(priority=HI)

        @pl.when(t + LEAD >= NO)
        def _():
            k_chunk_dyn(t + LEAD - NO).start(priority=HI)

        @pl.when(t + DEPTH < NO)
        def _():
            wo_chunk(t + DEPTH, 0).start(priority=LO)

        @pl.when(t + DEPTH >= NO)
        def _():
            v_chunk_dyn(t + DEPTH - NO).start(priority=LO)

    def kv_chunk_dyn(src, dst, sem, c):
        col = pl.multiple_of(c * CH, CH)
        return cp(src.at[0, :, pl.ds(SK - W + col, CH)], dst.at[0, :, pl.ds(col, CH)], sem.at[0])

    def k_chunk_dyn(c):
        return kv_chunk_dyn(k_hbm, kbuf, sem_k, c)

    def v_chunk_dyn(c):
        return kv_chunk_dyn(v_hbm, vbuf, sem_v, c)

    STEPS_PER_Q = NO // (H // 2)

    def a4_body(j, carry):
        for u in range(STEPS_PER_Q):
            wo_step(j * STEPS_PER_Q + u)
        q_piece(j)
        return carry
    lax.fori_loop(0, H // 2, a4_body, 0)

    acc_buf[...] = jnp.zeros_like(acc_buf)

    class Head:
        def __init__(self, h):
            self.h = h
            self.slot = h % R

        def qk(self, c0, n):
            for c in range(c0, c0 + n):
                s = jnp.dot(self.q8, kbuf[self.slot, :, c * CH:(c + 1) * CH],
                            preferred_element_type=jnp.float32)
                s_buf[c:c + 1, :] = s[0:1, :]

        def softmax(self):
            s = s_buf[...] * SCALE
            m = jnp.max(jnp.max(s, axis=0, keepdims=True), axis=1, keepdims=True)
            p = jnp.exp(s - m)
            self.l = jnp.sum(jnp.sum(p, axis=0, keepdims=True), axis=1, keepdims=True)
            s_buf[...] = p
            self.o = jnp.zeros((8, DH), jnp.float32)

        def pv(self, c0, n):
            for c in range(c0, c0 + n):
                p8 = _row8(s_buf[c:c + 1, :])
                self.o = self.o + lax.dot_general(
                    p8, vbuf[self.slot, :, c * CH:(c + 1) * CH],
                    (((1,), (1,)), ((), ())), preferred_element_type=jnp.float32)

        def finish(self):
            o8 = (self.o / self.l).astype(jnp.bfloat16)
            row = pl.multiple_of(self.h * DH, DH) if not isinstance(self.h, int) else self.h * DH
            acc_buf[...] += jnp.dot(o8, wo_buf[pl.ds(row, DH), :],
                                    preferred_element_type=jnp.float32)

        def start(self):
            wait_all(kbuf.at[self.slot], sem_k.at[self.slot])
            self.q8 = _row8(q_buf[pl.ds(self.h, 1), :])

        def piece(self, c, per_step=2):
            nq = NC // per_step
            if c == 0:
                self.start()
            if c < nq:
                self.qk(c * per_step, per_step)
            elif c < 2 * nq:
                if c == nq:
                    self.softmax()
                self.pv((c - nq) * per_step, per_step)
                if c == 2 * nq - 1:
                    self.finish()

    def period(p, last, compute):
        head = Head(p - 1) if compute else None
        for c in range(NC):
            v_chunk(p, c).wait()
            if c + LEAD < NC:
                k_chunk(p, c + LEAD).start(priority=HI)
            elif last:
                tail_chunk(c + LEAD - NC, 1).start(priority=HI)
            else:
                k_chunk(p + 1, c + LEAD - NC).start(priority=HI)
            if last:
                tail_chunk(c, 0).start(priority=LO)
            else:
                v_chunk(p + 1, c).start(priority=LO)
            if compute:
                head.piece(c)

    period(0, last=False, compute=False)
    for i in range(NO):
        wo_chunk(i, 1).wait()

    def b_body(p, carry):
        period(p, last=False, compute=True)
        return carry
    lax.fori_loop(1, H - 1, b_body, 0)
    period(H - 1, last=True, compute=True)

    def tail_step(t):
        tail_chunk(t, 0).wait()
        if t + LEAD < NT:
            tail_chunk(t + LEAD, 1).start(priority=HI)
        if t + DEPTH < NT:
            tail_chunk(t + DEPTH, 0).start(priority=LO)

    head = Head(H - 1)
    t = 0
    PER = 4
    for c in range(2 * NC // PER):
        tail_step(t)
        head.piece(c, per_step=PER)
        t += 1
    hres = x + acc_buf[0:1, :]
    xl = _layernorm(hres)
    xl8 = _row8(xl)
    wr = wr_buf[...].astype(jnp.float32).reshape(1, D)
    r = jnp.sum(xl.astype(jnp.bfloat16).astype(jnp.float32) * wr, axis=-1, keepdims=True)
    gate_r = jax.nn.sigmoid(r)
    while t < NG:
        tail_step(t)
        t += 1
    wait_all(wu_buf, sem_w.at[5])
    g = jnp.dot(xl8, wg_buf[...], preferred_element_type=jnp.float32)
    u = jnp.dot(xl8, wu_buf[...], preferred_element_type=jnp.float32)
    act = (g * jax.nn.sigmoid(g) * u).astype(jnp.bfloat16)
    y = jnp.zeros((8, D), jnp.float32)
    BLK = DN_BLK
    steps_per_blk = BLK // (2 * DN_ROWS)
    for b in range(F // BLK):
        for _ in range(steps_per_blk):
            tail_step(t)
            tail_chunk(t, 1).wait()
            t += 1
        y = y + jnp.dot(act[:, b * BLK:(b + 1) * BLK], wd_buf[b * BLK:(b + 1) * BLK, :],
                        preferred_element_type=jnp.float32)
    out = hres + (xl + y[0:1, :] * gate_r)
    o_ref[...] = out.astype(o_ref.dtype)


@jax.jit
def pallas_sequential_preLN__sliding_block_cached__moe_arch_mod__decode_kernel(
    A_x: jax.Array,
    A_k_cache: jax.Array,
    A_v_cache: jax.Array,
    A_wq: jax.Array,
    A_wo: jax.Array,
    B_x: jax.Array,
    B_w_r: jax.Array,
    B_w_gate: jax.Array,
    B_w_up: jax.Array,
    B_w_down: jax.Array,
):
    del B_x
    bf16 = jnp.bfloat16
    x2 = A_x.reshape(1, D)
    kt = jnp.swapaxes(A_k_cache, 2, 3).reshape(H, DH, SK)
    vt = jnp.swapaxes(A_v_cache, 2, 3).reshape(H, DH, SK)
    hbm = pl.BlockSpec(memory_space=pl.ANY)
    out = pl.pallas_call(
        _kernel,
        in_specs=[hbm] * 9,
        out_specs=pl.BlockSpec(memory_space=pltpu.VMEM),
        out_shape=jax.ShapeDtypeStruct((1, D), A_x.dtype),
        scratch_shapes=[
            pltpu.VMEM((R, DH, W), bf16),
            pltpu.VMEM((R, DH, W), bf16),
            pltpu.VMEM((D, H * DH), bf16),
            pltpu.VMEM((H * DH, D), bf16),
            pltpu.VMEM((D, F), bf16),
            pltpu.VMEM((D, F), bf16),
            pltpu.VMEM((F, D), bf16),
            pltpu.VMEM((1, D), bf16),
            pltpu.VMEM((D,), bf16),
            pltpu.VMEM((H, DH), jnp.float32),
            pltpu.VMEM((NC, CH), jnp.float32),
            pltpu.VMEM((8, D), jnp.float32),
            pltpu.SemaphoreType.DMA((R,)),
            pltpu.SemaphoreType.DMA((R,)),
            pltpu.SemaphoreType.DMA((8,)),
            pltpu.SemaphoreType.DMA((2 * (F // DN_BLK),)),
        ],
        compiler_params=pltpu.CompilerParams(
            vmem_limit_bytes=64 * 1024 * 1024,
            disable_bounds_checks=True,
        ),
    )(x2, kt, vt, A_wq, A_wo, B_w_r, B_w_gate, B_w_up, B_w_down)
    return out.reshape(1, 1, D)
```

```python
import functools

import jax
import jax.numpy as jnp
from jax import lax
import jax.experimental.pallas as pl
import jax.experimental.pallas.tpu as pltpu

D = 640
H = 32
DH = 192
SK = 32768
W = 4096
F = 1536
EPS = 1e-5
SCALE = 0.072265625

CH = 128
NC = W // CH
R = 4
DEPTH = NC
LEAD = 8
LO, HI = 1, 0

WQ_ROWS = 8
NQ = D // WQ_ROWS
WO_ROWS = 48
NO = H * DH // WO_ROWS // 2
NA = NQ + NO
G_ROWS = 16
NG = D // G_ROWS
DN_ROWS = 32
ND = F // DN_ROWS // 2
DN_BLK = 128
NT = NG + ND


def _layernorm(v):
    m = jnp.mean(v, axis=-1, keepdims=True)
    c = v - m
    var = jnp.mean(c * c, axis=-1, keepdims=True)
    return c / jnp.sqrt(var + EPS)


def _row8(v):
    return jnp.broadcast_to(v, (8, v.shape[1])).astype(jnp.bfloat16)


def _kernel(x_hbm, k_hbm, v_hbm, wq_hbm, wo_hbm, wr_hbm, wg_hbm, wu_hbm, wd_hbm,
            o_ref,
            kbuf, vbuf, wq_buf, wo_buf, wg_buf, wu_buf, wd_buf, x_buf, wr_buf,
            q_buf, s_buf, acc_buf,
            sem_k, sem_v, sem_w, sem_d):
    cp = pltpu.make_async_copy

    def rows(start, n, align):
        if isinstance(start, int):
            return pl.ds(start, n)
        return pl.ds(pl.multiple_of(start, align), n)

    def wq_chunk(i, half):
        r = rows(i * WQ_ROWS, WQ_ROWS, WQ_ROWS)
        c = pl.ds(half * (H * DH // 2), H * DH // 2)
        return cp(wq_hbm.at[r, c], wq_buf.at[r, c], sem_w.at[half])

    def wo_chunk(i, half):
        r = rows((i * 2 + half) * WO_ROWS, WO_ROWS, WO_ROWS)
        return cp(wo_hbm.at[r, :], wo_buf.at[r, :], sem_w.at[2 + half])

    def kv_chunk(src, dst, sem, h, c):
        slot = h % R
        return cp(src.at[h, :, pl.ds(SK - W + c * CH, CH)],
                  dst.at[slot, :, pl.ds(c * CH, CH)], sem.at[slot])

    def k_chunk(h, c):
        return kv_chunk(k_hbm, kbuf, sem_k, h, c)

    def v_chunk(h, c):
        return kv_chunk(v_hbm, vbuf, sem_v, h, c)

    def tail_chunk(i, half):
        if i < NG:
            r = pl.ds(i * G_ROWS, G_ROWS)
            if half == 0:
                return cp(wg_hbm.at[r, :], wg_buf.at[r, :], sem_w.at[4])
            return cp(wu_hbm.at[r, :], wu_buf.at[r, :], sem_w.at[5])
        j = i - NG
        r = pl.ds((2 * j + half) * DN_ROWS, DN_ROWS)
        return cp(wd_hbm.at[r, :], wd_buf.at[r, :],
                  sem_d.at[half * (F // DN_BLK) + (2 * j * DN_ROWS) // DN_BLK])

    def wait_all(buf, sem):
        cp(buf, buf, sem).wait()

    for i in range(LEAD):
        wq_chunk(i, 1).start(priority=HI)
        wq_chunk(i, 0).start(priority=LO)
    x_copy = cp(x_hbm, x_buf, sem_w.at[6])
    wr_copy = cp(wr_hbm, wr_buf, sem_w.at[7])
    x_copy.start(priority=HI)
    wr_copy.start(priority=HI)
    for i in range(LEAD, DEPTH):
        wq_chunk(i, 0).start(priority=LO)

    def a1_body(t, carry):
        wq_chunk(t, 0).wait()
        wq_chunk(t + LEAD, 1).start(priority=HI)
        wq_chunk(t + DEPTH, 0).start(priority=LO)
        return carry
    lax.fori_loop(0, NQ - DEPTH, a1_body, 0)

    def a2_body(t, carry):
        wq_chunk(t, 0).wait()
        wq_chunk(t + LEAD, 1).start(priority=HI)
        wo_chunk(t + DEPTH - NQ, 0).start(priority=LO)
        return carry
    lax.fori_loop(NQ - DEPTH, NQ - LEAD, a2_body, 0)

    def a3_body(t, carry):
        wq_chunk(t, 0).wait()
        wo_chunk(t + LEAD - NQ, 1).start(priority=HI)
        wo_chunk(t + DEPTH - NQ, 0).start(priority=LO)
        return carry
    lax.fori_loop(NQ - LEAD, NQ, a3_body, 0)

    x_copy.wait()
    wr_copy.wait()
    x = x_buf[...].astype(jnp.float32)
    xn8 = _row8(_layernorm(x))
    half_q = wq_buf.at[:, pl.ds(H * DH // 2, H * DH // 2)]
    cp(half_q, half_q, sem_w.at[1]).wait()

    def q_piece(j):
        col = pl.multiple_of(j * (2 * DH), 128)
        q2 = jnp.dot(xn8, wq_buf[:, pl.ds(col, 2 * DH)],
                     preferred_element_type=jnp.float32)
        q_buf[pl.ds(2 * j, 1), :] = q2[0:1, 0:DH]
        q_buf[pl.ds(2 * j + 1, 1), :] = q2[0:1, DH:2 * DH]

    def wo_step(t):
        wo_chunk(t, 0).wait()

        @pl.when(t + LEAD < NO)
        def _():
            wo_chunk(t + LEAD, 1).start(priority=HI)

        @pl.when(t + LEAD >= NO)
        def _():
            k_chunk_dyn(t + LEAD - NO).start(priority=HI)

        @pl.when(t + DEPTH < NO)
        def _():
            wo_chunk(t + DEPTH, 0).start(priority=LO)

        @pl.when(t + DEPTH >= NO)
        def _():
            v_chunk_dyn(t + DEPTH - NO).start(priority=LO)

    def kv_chunk_dyn(src, dst, sem, c):
        col = pl.multiple_of(c * CH, CH)
        return cp(src.at[0, :, pl.ds(SK - W + col, CH)], dst.at[0, :, pl.ds(col, CH)], sem.at[0])

    def k_chunk_dyn(c):
        return kv_chunk_dyn(k_hbm, kbuf, sem_k, c)

    def v_chunk_dyn(c):
        return kv_chunk_dyn(v_hbm, vbuf, sem_v, c)

    STEPS_PER_Q = NO // (H // 2)

    def a4_body(j, carry):
        for u in range(STEPS_PER_Q):
            wo_step(j * STEPS_PER_Q + u)
        q_piece(j)
        return carry
    lax.fori_loop(0, H // 2, a4_body, 0)

    acc_buf[...] = jnp.zeros_like(acc_buf)

    class Head:
        def __init__(self, h):
            self.h = h
            self.slot = h % R

        def qk(self, c0, n):
            for c in range(c0, c0 + n):
                s = jnp.dot(self.q8, kbuf[self.slot, :, c * CH:(c + 1) * CH],
                            preferred_element_type=jnp.float32)
                s_buf[c:c + 1, :] = s[0:1, :]

        def softmax(self):
            s = s_buf[...] * SCALE
            m = jnp.max(jnp.max(s, axis=0, keepdims=True), axis=1, keepdims=True)
            p = jnp.exp(s - m)
            self.l = jnp.sum(jnp.sum(p, axis=0, keepdims=True), axis=1, keepdims=True)
            s_buf[...] = p
            self.o = jnp.zeros((DH, CH), jnp.float32)

        def pv(self, c0, n):
            for c in range(c0, c0 + n):
                v = vbuf[self.slot, :, c * CH:(c + 1) * CH].astype(jnp.float32)
                self.o = self.o + v * s_buf[c:c + 1, :]

        def finish(self):
            o = jnp.sum(self.o.T, axis=0, keepdims=True) / self.l
            row = pl.multiple_of(self.h * DH, DH) if not isinstance(self.h, int) else self.h * DH
            acc_buf[...] += jnp.dot(_row8(o), wo_buf[pl.ds(row, DH), :],
                                    preferred_element_type=jnp.float32)

        def start(self):
            wait_all(kbuf.at[self.slot], sem_k.at[self.slot])
            self.q8 = _row8(q_buf[pl.ds(self.h, 1), :])

        def piece(self, c, per_step=2):
            nq = NC // per_step
            if c == 0:
                self.start()
            if c < nq:
                self.qk(c * per_step, per_step)
            elif c < 2 * nq:
                if c == nq:
                    self.softmax()
                self.pv((c - nq) * per_step, per_step)
                if c == 2 * nq - 1:
                    self.finish()

    def period(p, last, compute):
        head = Head(p - 1) if compute else None
        for c in range(NC):
            v_chunk(p, c).wait()
            if c + LEAD < NC:
                k_chunk(p, c + LEAD).start(priority=HI)
            elif last:
                tail_chunk(c + LEAD - NC, 1).start(priority=HI)
            else:
                k_chunk(p + 1, c + LEAD - NC).start(priority=HI)
            if last:
                tail_chunk(c, 0).start(priority=LO)
            else:
                v_chunk(p + 1, c).start(priority=LO)
            if compute:
                head.piece(c)

    period(0, last=False, compute=False)
    for i in range(NO):
        wo_chunk(i, 1).wait()

    def b_body(p, carry):
        period(p, last=False, compute=True)
        return carry
    lax.fori_loop(1, H - 1, b_body, 0)
    period(H - 1, last=True, compute=True)

    def tail_step(t):
        tail_chunk(t, 0).wait()
        if t + LEAD < NT:
            tail_chunk(t + LEAD, 1).start(priority=HI)
        if t + DEPTH < NT:
            tail_chunk(t + DEPTH, 0).start(priority=LO)

    head = Head(H - 1)
    t = 0
    PER = 4
    for c in range(2 * NC // PER):
        tail_step(t)
        head.piece(c, per_step=PER)
        t += 1
    hres = x + acc_buf[0:1, :]
    xl = _layernorm(hres)
    xl8 = _row8(xl)
    wr = wr_buf[...].astype(jnp.float32).reshape(1, D)
    r = jnp.sum(xl.astype(jnp.bfloat16).astype(jnp.float32) * wr, axis=-1, keepdims=True)
    gate_r = jax.nn.sigmoid(r)
    while t < NG:
        tail_step(t)
        t += 1
    wait_all(wu_buf, sem_w.at[5])
    g = jnp.dot(xl8, wg_buf[...], preferred_element_type=jnp.float32)
    u = jnp.dot(xl8, wu_buf[...], preferred_element_type=jnp.float32)
    act = (g * jax.nn.sigmoid(g) * u).astype(jnp.bfloat16)
    y = jnp.zeros((8, D), jnp.float32)
    BLK = DN_BLK
    steps_per_blk = BLK // (2 * DN_ROWS)
    for b in range(F // BLK):
        for _ in range(steps_per_blk):
            tail_step(t)
            tail_chunk(t, 1).wait()
            t += 1
        y = y + jnp.dot(act[:, b * BLK:(b + 1) * BLK], wd_buf[b * BLK:(b + 1) * BLK, :],
                        preferred_element_type=jnp.float32)
    out = hres + (xl + y[0:1, :] * gate_r)
    o_ref[...] = out.astype(o_ref.dtype)


@jax.jit
def pallas_sequential_preLN__sliding_block_cached__moe_arch_mod__decode_kernel(
    A_x: jax.Array,
    A_k_cache: jax.Array,
    A_v_cache: jax.Array,
    A_wq: jax.Array,
    A_wo: jax.Array,
    B_x: jax.Array,
    B_w_r: jax.Array,
    B_w_gate: jax.Array,
    B_w_up: jax.Array,
    B_w_down: jax.Array,
):
    del B_x
    bf16 = jnp.bfloat16
    x2 = A_x.reshape(1, D)
    kt = jnp.swapaxes(A_k_cache, 2, 3).reshape(H, DH, SK)
    vt = jnp.swapaxes(A_v_cache, 2, 3).reshape(H, DH, SK)
    hbm = pl.BlockSpec(memory_space=pl.ANY)
    out = pl.pallas_call(
        _kernel,
        in_specs=[hbm] * 9,
        out_specs=pl.BlockSpec(memory_space=pltpu.VMEM),
        out_shape=jax.ShapeDtypeStruct((1, D), A_x.dtype),
        scratch_shapes=[
            pltpu.VMEM((R, DH, W), bf16),
            pltpu.VMEM((R, DH, W), bf16),
            pltpu.VMEM((D, H * DH), bf16),
            pltpu.VMEM((H * DH, D), bf16),
            pltpu.VMEM((D, F), bf16),
            pltpu.VMEM((D, F), bf16),
            pltpu.VMEM((F, D), bf16),
            pltpu.VMEM((1, D), bf16),
            pltpu.VMEM((D,), bf16),
            pltpu.VMEM((H, DH), jnp.float32),
            pltpu.VMEM((NC, CH), jnp.float32),
            pltpu.VMEM((8, D), jnp.float32),
            pltpu.SemaphoreType.DMA((R,)),
            pltpu.SemaphoreType.DMA((R,)),
            pltpu.SemaphoreType.DMA((8,)),
            pltpu.SemaphoreType.DMA((2 * (F // DN_BLK),)),
        ],
        compiler_params=pltpu.CompilerParams(
            vmem_limit_bytes=64 * 1024 * 1024,
            disable_bounds_checks=True,
        ),
    )(x2, kt, vt, A_wq, A_wo, B_w_r, B_w_gate, B_w_up, B_w_down)
    return out.reshape(1, 1, D)
```

```python
import functools

import jax
import jax.numpy as jnp
from jax import lax
import jax.experimental.pallas as pl
import jax.experimental.pallas.tpu as pltpu

D = 640
H = 32
DH = 192
SK = 32768
W = 4096
F = 1536
EPS = 1e-5
SCALE = 0.072265625

LO, HI = 1, 0
CH = 128
NC = W // CH
HS = 2
RH = DH // HS
NS = NC * HS
RK = 4
RV = 8
DEPTH = 48
LEAD = 20
LEAD_W = 8

NPQ = 5
WQ_ROWS = 160
WQ_RB = D // WQ_ROWS
NQT = H * DH // 128
NWQ = NQT * WQ_RB
WQ_GT = 4
WO_ROWS = 32
NWO = H * DH // WO_ROWS
WO_G = 32
G_ROWS = 16
NG = D // G_ROWS
GB = 128
DN_ROWS = 32
ND = F // DN_ROWS // 2
DN_BLK = 128
NT = NG + ND

T_K0 = NPQ * NS
T_WO = H * NS
T_TAIL = T_WO + NWO
T_END = T_TAIL + NT
HI_K0 = NWQ
HI_SLOW = NWQ + (T_WO - T_K0)
HI_TAIL = NWQ + H * NS
HI_END = HI_TAIL + NT


def _hi_due(i):
    if i < HI_K0:
        return (i * T_K0) // NWQ
    if i < HI_SLOW:
        return T_K0 + (i - HI_K0)
    if i < HI_TAIL:
        return T_WO + -(-((i - HI_SLOW) * NWO) // (HI_TAIL - HI_SLOW))
    return T_TAIL + (i - HI_TAIL)


def _head_sched(kind):
    if kind == "fine":
        qk = {2 * i: (2 * i, 2) for i in range(16)}
        n = [2] * 2 + [1] * 28
        pv = {33 + i: (sum(n[:i]), n[i]) for i in range(30)}
        return dict(qk=qk, sm=32, pv=pv, fin=63)
    if kind == "coarse":
        qk = {2 * i: (4 * i, 4) for i in range(8)}
        n = [3] * 4 + [2] * 10
        pv = {17 + i: (sum(n[:i]), n[i]) for i in range(14)}
        return dict(qk=qk, sm=16, pv=pv, fin=31)
    assert kind == "last"
    qk = {i: (4 * i, 4) for i in range(8)}
    pv = {9 + i: (4 * i, 4) for i in range(8)}
    return dict(qk=qk, sm=8, pv=pv, fin=17)


def _layernorm(v):
    m = jnp.mean(v, axis=-1, keepdims=True)
    c = v - m
    var = jnp.mean(c * c, axis=-1, keepdims=True)
    return c / jnp.sqrt(var + EPS)


def _row8(v):
    return jnp.broadcast_to(v, (8, v.shape[1])).astype(jnp.bfloat16)


def _kernel(x_hbm, k_hbm, v_hbm, wq_hbm, wo_hbm, wr_hbm, wg_hbm, wu_hbm, wd_hbm,
            o_ref,
            kbuf, vbuf, wq_buf, wo_buf, wg_buf, wu_buf, wd_buf, x_buf, wr_buf,
            xn_buf, qf_buf, q_buf, s_buf, o_buf, acc_buf,
            sem_k, sem_v, sem_x, sem_q, sem_o, sem_g, sem_d):
    cp = pltpu.make_async_copy
    f32 = jnp.float32

    def wq_chunk(i):
        j, rb = i // WQ_RB, i % WQ_RB
        r, c = pl.ds(rb * WQ_ROWS, WQ_ROWS), pl.ds(j * 128, 128)
        return cp(wq_hbm.at[r, c], wq_buf.at[r, c], sem_q.at[j // WQ_GT])

    def wo_chunk(k):
        r = pl.ds(k * WO_ROWS, WO_ROWS)
        return cp(wo_hbm.at[r, :], wo_buf.at[r, :], sem_o.at[k // WO_G])

    def kv_chunk(src, dst, sem, slot, h, w):
        c, r = w // HS, w % HS
        rows = pl.ds(r * RH, RH)
        return cp(src.at[h, rows, pl.ds(SK - W + c * CH, CH)],
                  dst.at[slot, rows, pl.ds(c * CH, CH)], sem.at[slot])

    def k_chunk(h, w):
        return kv_chunk(k_hbm, kbuf, sem_k, h % RK, h, w)

    def v_chunk(h, w):
        return kv_chunk(v_hbm, vbuf, sem_v, h % RV, h, w)

    def tail_chunk(i, hi):
        if i < NG:
            r = pl.ds(i * G_ROWS, G_ROWS)
            b = (i * G_ROWS) // GB
            if hi:
                return cp(wu_hbm.at[r, :], wu_buf.at[r, :], sem_g.at[D // GB + b])
            return cp(wg_hbm.at[r, :], wg_buf.at[r, :], sem_g.at[b])
        j = i - NG
        r = pl.ds((2 * j + hi) * DN_ROWS, DN_ROWS)
        b = (2 * j * DN_ROWS) // DN_BLK
        return cp(wd_hbm.at[r, :], wd_buf.at[r, :], sem_d.at[hi * (F // DN_BLK) + b])

    def lo_chunk(t):
        if t < T_WO:
            return v_chunk(t // NS, t % NS)
        if t < T_TAIL:
            return wo_chunk(t - T_WO)
        return tail_chunk(t - T_TAIL, 0)

    def hi_chunk(i):
        if i < HI_K0:
            return wq_chunk(i)
        if i < HI_TAIL:
            return k_chunk((i - HI_K0) // NS, (i - HI_K0) % NS)
        return tail_chunk(i - HI_TAIL, 1)

    def wait_all(buf, sem):
        cp(buf, buf, sem).wait()

    hi_issue = {}
    for i in range(HI_END):
        due = _hi_due(i)
        hi_issue.setdefault(max(due - (LEAD if due <= T_WO else LEAD_W), -1), []).append(i)

    def dma_step(t):
        lo_chunk(t).wait()
        for i in hi_issue.get(t, []):
            hi_chunk(i).start(priority=HI)
        if t + DEPTH < T_END:
            lo_chunk(t + DEPTH).start(priority=LO)

    first_hi = hi_issue.get(-1, [])
    for n, i in enumerate(first_hi):
        hi_chunk(i).start(priority=HI)
        lo_chunk(n).start(priority=LO)
    x_copy = cp(x_hbm, x_buf, sem_x.at[0])
    wr_copy = cp(wr_hbm, wr_buf, sem_x.at[1])
    x_copy.start(priority=HI)
    wr_copy.start(priority=HI)
    for t in range(len(first_hi), DEPTH):
        lo_chunk(t).start(priority=LO)

    def ln_x():
        x_copy.wait()
        wr_copy.wait()
        xn_buf[...] = _row8(_layernorm(x_buf[...].astype(f32)))
        acc_buf[...] = jnp.zeros_like(acc_buf)

    def q_tile(j):
        if j % WQ_GT == 0:
            wait_all(wq_buf.at[:, pl.ds(j * 128, WQ_GT * 128)], sem_q.at[j // WQ_GT])
        cols = slice(j * 128, (j + 1) * 128)
        qf_buf[:, cols] = jnp.dot(xn_buf[...], wq_buf[:, cols], preferred_element_type=f32)

    def q_pair(j):
        c0 = j * 2 * DH
        q_buf[2 * j:2 * j + 1, :] = qf_buf[0:1, c0:c0 + DH]
        q_buf[2 * j + 1:2 * j + 2, :] = qf_buf[0:1, c0 + DH:c0 + 2 * DH]

    class Head:
        def __init__(self, h, kind):
            self.h = h
            self.plan = _head_sched(kind)
            self.len = self.plan["fin"] + 1

        def wait_k(self):
            slot = self.h % RK
            wait_all(kbuf.at[slot], sem_k.at[slot])

        def piece(self, c):
            plan, h = self.plan, self.h
            if c == 0:
                self.q8 = _row8(q_buf[pl.ds(h, 1), :])
            if c in plan["qk"]:
                c0, n = plan["qk"][c]
                for j in range(c0, c0 + n):
                    s = jnp.dot(self.q8, kbuf[h % RK, :, j * CH:(j + 1) * CH],
                                preferred_element_type=f32)
                    s_buf[j:j + 1, :] = s[0:1, :]
            if c == plan["sm"]:
                s = s_buf[...] * SCALE
                m = jnp.max(jnp.max(s, axis=0, keepdims=True), axis=1, keepdims=True)
                p = jnp.exp(s - m)
                self.l = jnp.sum(jnp.sum(p, axis=0, keepdims=True), axis=1, keepdims=True)
                s_buf[...] = p
                self.o = jnp.zeros((DH, CH), f32)
            if c in plan["pv"]:
                c0, n = plan["pv"][c]
                for j in range(c0, c0 + n):
                    v = vbuf[h % RV, :, j * CH:(j + 1) * CH].astype(f32)
                    self.o = self.o + v * s_buf[j:j + 1, :]
            if c == plan["fin"]:
                o_buf[pl.ds(h, 1), :] = jnp.sum(self.o.T, axis=0, keepdims=True) / self.l

    def wo_apply(h0, h1):
        o = [o_buf[h:h + 1, :] for h in range(h0, h1)]
        o = jnp.concatenate(o, axis=1) if len(o) > 1 else o[0]
        acc_buf[...] += jnp.dot(_row8(o), wo_buf[h0 * DH:h1 * DH, :], preferred_element_type=f32)

    early = {8 * HS: [ln_x]}
    tq = 10 * HS
    for j in range(NQT):
        last = (j // WQ_GT + 1) * WQ_GT * WQ_RB - 1
        tq = max(tq + HS, _hi_due(last) + 2 * HS)
        early.setdefault(tq, []).append(functools.partial(q_tile, j))
        if j % 3 == 2:
            tq += HS
            early.setdefault(tq, []).append(functools.partial(q_pair, j // 3))
    assert tq < (NPQ + 1) * NS
    for t in range((NPQ + 1) * NS):
        dma_step(t)
        for fn in early.get(t, []):
            fn()

    def period(P, carry):
        head = Head(P - NPQ - 1, "fine")
        for c in range(NS):
            v_chunk(P, c).wait()
            ch = c + LEAD
            k_chunk(P - NPQ + ch // NS, ch % NS).start(priority=HI)
            cl = c + DEPTH
            v_chunk(P + cl // NS, cl % NS).start(priority=LO)
            if c == 0:
                head.wait_k()
            head.piece(c)
        return carry

    p_end = H - 1
    lax.fori_loop(NPQ + 1, p_end, period, 0)

    def head_start(h):
        return _hi_due(HI_K0 + (h + 1) * NS - 1) + 1

    work = {}

    def add(t, fn):
        work.setdefault(t, []).append(fn)

    t_static = p_end * NS
    h_first = p_end - NPQ - 1
    heads = {}
    for h in range(h_first, H):
        kind = "last" if h == H - 1 else ("fine" if head_start(h) < T_WO else "coarse")
        heads[h] = Head(h, kind)
    busy = set()
    for h, head in heads.items():
        s0 = head_start(h)
        assert s0 >= t_static
        add(s0, head.wait_k)
        for c in range(head.len):
            add(s0 + c, functools.partial(head.piece, c))
        busy.update(s0 + c for c in list(head.plan["qk"]) + [head.plan["sm"], head.plan["fin"]])
    t_mid = head_start(H - 1) + heads[H - 1].len

    def wo_ready(h):
        return T_WO + (((h + 1) * DH - 1) // WO_ROWS // WO_G + 1) * WO_G

    h = 0
    while h < H - 1:
        h1 = h + 1
        while h1 < H - 1 and wo_ready(h1) == wo_ready(h):
            h1 += 1
        done = head_start(h1 - 1) + (heads[h1 - 1].len if h1 - 1 in heads else NS)
        t = [t for t in range(max(wo_ready(h), done), t_mid) if t not in busy][0]
        busy.add(t)
        add(t, functools.partial(wo_apply, h, h1))
        h = h1

    st = {}

    def mid():
        wo_apply(H - 1, H)
        st["h"] = x_buf[...].astype(f32) + acc_buf[0:1, :]
        st["xl"] = _layernorm(st["h"])
        st["xl8"] = _row8(st["xl"])
        wr = wr_buf[...].astype(f32).reshape(1, D)
        r = jnp.sum(st["xl"].astype(jnp.bfloat16).astype(f32) * wr, axis=-1, keepdims=True)
        st["gate_r"] = jax.nn.sigmoid(r)

    def gu_block(b):
        wait_all(wu_buf.at[pl.ds(b * GB, GB), :], sem_g.at[D // GB + b])
        rows = slice(b * GB, (b + 1) * GB)
        g = jnp.dot(st["xl8"][:, rows], wg_buf[rows, :], preferred_element_type=f32)
        u = jnp.dot(st["xl8"][:, rows], wu_buf[rows, :], preferred_element_type=f32)
        st["g"] = g if b == 0 else st["g"] + g
        st["u"] = u if b == 0 else st["u"] + u
        if b == D // GB - 1:
            g, u = st["g"], st["u"]
            st["act"] = (g * jax.nn.sigmoid(g) * u).astype(jnp.bfloat16)
            st["y"] = jnp.zeros((8, D), f32)

    def dn_block(b):
        for j in range(2 * b, 2 * b + 2):
            tail_chunk(NG + j, 1).wait()
        rows = slice(b * DN_BLK, (b + 1) * DN_BLK)
        st["y"] = st["y"] + jnp.dot(st["act"][:, rows], wd_buf[rows, :],
                                    preferred_element_type=f32)

    add(t_mid, mid)
    t = t_mid
    for b in range(D // GB):
        t = max(t + 1, T_TAIL + (b + 1) * (GB // G_ROWS) - 1)
        add(t, functools.partial(gu_block, b))
    for b in range(F // DN_BLK):
        t = max(t, T_TAIL + NG + 2 * b + 1)
        add(t, functools.partial(dn_block, b))
    assert max(work) < T_END

    for t in range(t_static, T_END):
        dma_step(t)
        for fn in work.get(t, []):
            fn()

    out = st["h"] + (st["xl"] + st["y"][0:1, :] * st["gate_r"])
    o_ref[...] = out.astype(o_ref.dtype)


@jax.jit
def pallas_sequential_preLN__sliding_block_cached__moe_arch_mod__decode_kernel(
    A_x: jax.Array,
    A_k_cache: jax.Array,
    A_v_cache: jax.Array,
    A_wq: jax.Array,
    A_wo: jax.Array,
    B_x: jax.Array,
    B_w_r: jax.Array,
    B_w_gate: jax.Array,
    B_w_up: jax.Array,
    B_w_down: jax.Array,
):
    del B_x
    bf16, f32 = jnp.bfloat16, jnp.float32
    x2 = A_x.reshape(1, D)
    kt = jnp.swapaxes(A_k_cache, 2, 3).reshape(H, DH, SK)
    vt = jnp.swapaxes(A_v_cache, 2, 3).reshape(H, DH, SK)
    hbm = pl.BlockSpec(memory_space=pl.ANY)
    dma = pltpu.SemaphoreType.DMA
    out = pl.pallas_call(
        _kernel,
        in_specs=[hbm] * 9,
        out_specs=pl.BlockSpec(memory_space=pltpu.VMEM),
        out_shape=jax.ShapeDtypeStruct((1, D), A_x.dtype),
        scratch_shapes=[
            pltpu.VMEM((RK, DH, W), bf16),
            pltpu.VMEM((RV, DH, W), bf16),
            pltpu.VMEM((D, H * DH), bf16),
            pltpu.VMEM((H * DH, D), bf16),
            pltpu.VMEM((D, F), bf16),
            pltpu.VMEM((D, F), bf16),
            pltpu.VMEM((F, D), bf16),
            pltpu.VMEM((1, D), bf16),
            pltpu.VMEM((D,), bf16),
            pltpu.VMEM((8, D), bf16),
            pltpu.VMEM((8, H * DH), f32),
            pltpu.VMEM((H, DH), f32),
            pltpu.VMEM((NC, CH), f32),
            pltpu.VMEM((H, DH), f32),
            pltpu.VMEM((8, D), f32),
            dma((RK,)),
            dma((RV,)),
            dma((2,)),
            dma((NQT // WQ_GT,)),
            dma((NWO // WO_G,)),
            dma((2 * (D // GB),)),
            dma((2 * (F // DN_BLK),)),
        ],
        compiler_params=pltpu.CompilerParams(
            vmem_limit_bytes=64 * 1024 * 1024,
            disable_bounds_checks=True,
            disable_semaphore_checks=True,
        ),
    )(x2, kt, vt, A_wq, A_wo, B_w_r, B_w_gate, B_w_up, B_w_down)
    return out.reshape(1, 1, D)
```

```python
import functools

import jax
import jax.numpy as jnp
from jax import lax
import jax.experimental.pallas as pl
import jax.experimental.pallas.tpu as pltpu

D = 640
H = 32
DH = 192
SK = 32768
W = 4096
F = 1536
EPS = 1e-5
SCALE = 0.072265625

LO, HI = 1, 0
CH = 128
NC = W // CH
HS = 2
RH = DH // HS
NS = NC * HS
RK = 4
RV = 8
DEPTH = 48
LEAD = 20
DEPTH_W = 24
LEAD_W = 10
K_ROT = 60

NPQ = 5
WQ_G, WQ_R = 10, 64
NQT = H * DH // 128
NWQ = (WQ_R // 8) * NQT
WO_G, WO_R = 12, 512
NWO = (WO_R // 8) * (D // 128)
assert NWO == NPQ * NS
WO_STEP = 44
G_ROWS = 16
NG = D // G_ROWS
GB = 128
DN_ROWS = 32
ND = F // DN_ROWS // 2
DN_BLK = 128
NT = NG + ND

T_K0 = NPQ * NS
T_TAIL = (H + NPQ) * NS
T_END = T_TAIL + NT
HI_K0 = NWQ
HI_TAIL = NWQ + H * NS
HI_END = HI_TAIL + NT


def _hi_due(i):
    if i < HI_K0:
        return (i * T_K0) // NWQ
    return T_K0 + (i - HI_K0)


def _issue_step(due, n_short, n_long):
    if due < T_TAIL:
        return max(due - n_short, -1)
    back = due - T_TAIL - n_long
    return T_TAIL + back if back >= 0 else T_TAIL + 2 * back


def _head_sched(kind):
    if kind == "fine":
        qk = {2 * i: (2 * i, 2) for i in range(16)}
        n = [2] * 2 + [1] * 28
        pv = {33 + i: (sum(n[:i]), n[i]) for i in range(30)}
        return dict(qk=qk, sm=32, pv=pv, fin=63)
    assert kind == "last"
    qk = {i: (4 * i, 4) for i in range(8)}
    pv = {9 + i: (4 * i, 4) for i in range(8)}
    return dict(qk=qk, sm=8, pv=pv, fin=17)


def _layernorm(v):
    m = jnp.mean(v, axis=-1, keepdims=True)
    c = v - m
    var = jnp.mean(c * c, axis=-1, keepdims=True)
    return c / jnp.sqrt(var + EPS)


def _row8(v):
    return jnp.broadcast_to(v, (8, v.shape[1])).astype(jnp.bfloat16)


def _kernel(x_hbm, k_hbm, v_hbm, wq_hbm, wo_hbm, wr_hbm, wg_hbm, wu_hbm, wd_hbm,
            o_ref,
            kbuf, vbuf, wq_buf, wo_buf, wg_buf, wu_buf, wd_buf, x_buf, wr_buf,
            xn_buf, q_buf, s_buf, o_buf, acc_buf,
            sem_k, sem_v, sem_x, sem_q, sem_o, sem_g, sem_d):
    cp = pltpu.make_async_copy
    f32 = jnp.float32

    def wq_chunk(i):
        r, j = pl.ds((i // NQT) * 8, 8), i % NQT
        c = pl.ds(j * 128, 128)
        return cp(wq_hbm.at[:, r, c], wq_buf.at[:, r, c], sem_q.at[j // 3])

    def wo_chunk(k):
        r, c = pl.ds((k // 5) * 8, 8), pl.ds((k % 5) * 128, 128)
        return cp(wo_hbm.at[:, r, c], wo_buf.at[:, r, c], sem_o.at[0])

    def kv_chunk(src, dst, sem, slot, h, w):
        c, r = w // HS, w % HS
        rows = pl.ds(r * RH, RH)
        return cp(src.at[h, rows, pl.ds(SK - W + c * CH, CH)],
                  dst.at[slot, rows, pl.ds(c * CH, CH)], sem.at[slot])

    def k_chunk(h, w):
        return kv_chunk(k_hbm, kbuf, sem_k, h % RK, h, (w + K_ROT) % NS)

    def v_chunk(h, w):
        return kv_chunk(v_hbm, vbuf, sem_v, h % RV, h, w)

    def tail_chunk(i, hi):
        if i < NG:
            r = pl.ds(i * G_ROWS, G_ROWS)
            b = (i * G_ROWS) // GB
            if hi:
                return cp(wu_hbm.at[r, :], wu_buf.at[r, :], sem_g.at[D // GB + b])
            return cp(wg_hbm.at[r, :], wg_buf.at[r, :], sem_g.at[b])
        j = i - NG
        r = pl.ds((2 * j + hi) * DN_ROWS, DN_ROWS)
        b = (2 * j * DN_ROWS) // DN_BLK
        return cp(wd_hbm.at[r, :], wd_buf.at[r, :], sem_d.at[hi * (F // DN_BLK) + b])

    def lo_chunk(t):
        p, w = t // NS, t % NS
        if p < NPQ:
            return v_chunk(p, w)
        if p < 2 * NPQ:
            return wo_chunk(t - NPQ * NS)
        if t < T_TAIL:
            return v_chunk(p - NPQ, w)
        return tail_chunk(t - T_TAIL, 0)

    def hi_chunk(i):
        if i < HI_K0:
            return wq_chunk(i)
        if i < HI_TAIL:
            return k_chunk((i - HI_K0) // NS, (i - HI_K0) % NS)
        return tail_chunk(i - HI_TAIL, 1)

    def wait_all(buf, sem):
        cp(buf, buf, sem).wait()

    hi_issue, lo_issue = {}, {}
    for i in range(HI_END):
        hi_issue.setdefault(_issue_step(_hi_due(i), LEAD, LEAD_W), []).append(i)
    for t in range(T_END):
        lo_issue.setdefault(_issue_step(t, DEPTH, DEPTH_W), []).append(t)

    def dma_step(t):
        lo_chunk(t).wait()
        for i in hi_issue.get(t, []):
            hi_chunk(i).start(priority=HI)
        for u in lo_issue.get(t, []):
            lo_chunk(u).start(priority=LO)

    first_hi, first_lo = hi_issue[-1], lo_issue[-1]
    for n, i in enumerate(first_hi):
        hi_chunk(i).start(priority=HI)
        lo_chunk(first_lo[n]).start(priority=LO)
    x_copy = cp(x_hbm, x_buf, sem_x.at[0])
    wr_copy = cp(wr_hbm, wr_buf, sem_x.at[1])
    x_copy.start(priority=HI)
    wr_copy.start(priority=HI)
    for u in first_lo[len(first_hi):]:
        lo_chunk(u).start(priority=LO)

    def ln_x():
        x_copy.wait()
        wr_copy.wait()
        xn_buf[...] = _row8(_layernorm(x_buf[...].astype(f32)))
        acc_buf[...] = jnp.zeros_like(acc_buf)

    def q_pair(j):
        wait_all(wq_buf.at[:, :, pl.ds(j * 2 * DH, 2 * DH)], sem_q.at[j])
        w = wq_buf[:, :, j * 2 * DH:(j + 1) * 2 * DH].reshape(D, 2 * DH)
        q2 = jnp.dot(xn_buf[...], w, preferred_element_type=f32)
        q_buf[2 * j:2 * j + 1, :] = q2[0:1, 0:DH]
        q_buf[2 * j + 1:2 * j + 2, :] = q2[0:1, DH:2 * DH]

    class Head:
        def __init__(self, h, kind):
            self.h = h
            self.plan = _head_sched(kind)
            self.len = self.plan["fin"] + 1

        def wait_k(self):
            slot = self.h % RK
            wait_all(kbuf.at[slot], sem_k.at[slot])

        def piece(self, c):
            plan, h = self.plan, self.h
            if c == 0:
                self.q8 = _row8(q_buf[pl.ds(h, 1), :])
            if c in plan["qk"]:
                c0, n = plan["qk"][c]
                for j in range(c0, c0 + n):
                    s = jnp.dot(self.q8, kbuf[h % RK, :, j * CH:(j + 1) * CH],
                                preferred_element_type=f32)
                    s_buf[j:j + 1, :] = s[0:1, :]
            if c == plan["sm"]:
                s = s_buf[...] * SCALE
                m = jnp.max(jnp.max(s, axis=0, keepdims=True), axis=1, keepdims=True)
                p = jnp.exp(s - m)
                self.l = jnp.sum(jnp.sum(p, axis=0, keepdims=True), axis=1, keepdims=True)
                s_buf[...] = p
                self.o = jnp.zeros((DH, CH), f32)
            if c in plan["pv"]:
                c0, n = plan["pv"][c]
                for j in range(c0, c0 + n):
                    v = vbuf[h % RV, :, j * CH:(j + 1) * CH].astype(f32)
                    self.o = self.o + v * s_buf[j:j + 1, :]
            if c == plan["fin"]:
                o_buf[pl.ds(h, 1), :] = jnp.sum(self.o.T, axis=0, keepdims=True) / self.l

    def wo_rows(h):
        blocks = []
        for i in range(DH // 64):
            b = h * (DH // 64) + i
            if isinstance(b, int):
                blocks.append(wo_buf[b // 8, (b % 8) * 64:(b % 8 + 1) * 64, :])
            else:
                blocks.append(wo_buf[b // 8, pl.ds(pl.multiple_of((b % 8) * 64, 64), 64), :])
        return blocks

    def wo_apply(h0, h1=None):
        if h1 is None:
            o, w = o_buf[pl.ds(h0, 1), :], wo_rows(h0)
        else:
            o = jnp.concatenate([o_buf[h:h + 1, :] for h in range(h0, h1)], axis=1)
            w = sum((wo_rows(h) for h in range(h0, h1)), [])
        acc_buf[...] += jnp.dot(_row8(o), jnp.concatenate(w, axis=0), preferred_element_type=f32)

    work = {}

    def add(t, fn):
        work.setdefault(t, []).append(fn)

    def add_head(head, s0):
        add(s0, head.wait_k)
        for c in range(head.len):
            add(s0 + c, functools.partial(head.piece, c))

    def run_static(t0, t1):
        for t in range(t0, t1):
            dma_step(t)
            for fn in work.get(t, []):
                fn()

    add(8 * HS, ln_x)
    t = 0
    for j in range(H // 2):
        last = (WQ_R // 8 - 1) * NQT + 3 * j + 2
        t = max(t + 4, _hi_due(last) + 2)
        add(t, functools.partial(q_pair, j))
    assert t < (NPQ + 1) * NS
    p_loop = 2 * NPQ
    for h in range(p_loop - NPQ - 1):
        add_head(Head(h, "fine"), (h + NPQ + 1) * NS)
    run_static(0, p_loop * NS)
    wo_apply(0, p_loop - NPQ - 2)

    def period(P, carry):
        head = Head(P - NPQ - 1, "fine")
        for c in range(NS):
            v_chunk(P - NPQ, c).wait()
            ch = c + LEAD
            k_chunk(P - NPQ + ch // NS, ch % NS).start(priority=HI)
            cl = c + DEPTH
            v_chunk(P - NPQ + cl // NS, cl % NS).start(priority=LO)
            if c == 0:
                head.wait_k()
            head.piece(c)
            if c == WO_STEP:
                wo_apply(P - NPQ - 2)
        return carry

    p_end = H + NPQ - 1
    lax.fori_loop(p_loop, p_end, period, 0)

    work.clear()
    t_static = p_end * NS
    assert _issue_step(T_TAIL, DEPTH, DEPTH_W) >= t_static
    add_head(Head(H - 2, "fine"), t_static)
    add(t_static + WO_STEP, functools.partial(wo_apply, H - 3))
    last_head = Head(H - 1, "last")
    add_head(last_head, T_TAIL)
    add(T_TAIL + last_head.plan["sm"], functools.partial(wo_apply, H - 2))
    t_mid = T_TAIL + last_head.len
    st = {}

    def mid():
        wo_apply(H - 1)
        st["h"] = x_buf[...].astype(f32) + acc_buf[0:1, :]
        st["xl"] = _layernorm(st["h"])
        st["xl8"] = _row8(st["xl"])
        wr = wr_buf[...].astype(f32).reshape(1, D)
        r = jnp.sum(st["xl"].astype(jnp.bfloat16).astype(f32) * wr, axis=-1, keepdims=True)
        st["gate_r"] = jax.nn.sigmoid(r)

    def gu_block(b):
        wait_all(wu_buf.at[pl.ds(b * GB, GB), :], sem_g.at[D // GB + b])
        rows = slice(b * GB, (b + 1) * GB)
        g = jnp.dot(st["xl8"][:, rows], wg_buf[rows, :], preferred_element_type=f32)
        u = jnp.dot(st["xl8"][:, rows], wu_buf[rows, :], preferred_element_type=f32)
        st["g"] = g if b == 0 else st["g"] + g
        st["u"] = u if b == 0 else st["u"] + u
        if b == D // GB - 1:
            g, u = st["g"], st["u"]
            st["act"] = (g * jax.nn.sigmoid(g) * u).astype(jnp.bfloat16)
            st["y"] = jnp.zeros((8, D), f32)

    def dn_block(b):
        for j in range(2 * b, 2 * b + 2):
            tail_chunk(NG + j, 1).wait()
        rows = slice(b * DN_BLK, (b + 1) * DN_BLK)
        st["y"] = st["y"] + jnp.dot(st["act"][:, rows], wd_buf[rows, :],
                                    preferred_element_type=f32)

    add(t_mid, mid)
    t = t_mid
    for b in range(D // GB):
        t = max(t + 1, T_TAIL + (b + 1) * (GB // G_ROWS) - 1)
        add(t, functools.partial(gu_block, b))
    for b in range(F // DN_BLK):
        t = max(t, T_TAIL + NG + 2 * b + 1)
        add(t, functools.partial(dn_block, b))
    assert max(work) < T_END
    run_static(t_static, T_END)

    out = st["h"] + (st["xl"] + st["y"][0:1, :] * st["gate_r"])
    o_ref[...] = out.astype(o_ref.dtype)


@jax.jit
def pallas_sequential_preLN__sliding_block_cached__moe_arch_mod__decode_kernel(
    A_x: jax.Array,
    A_k_cache: jax.Array,
    A_v_cache: jax.Array,
    A_wq: jax.Array,
    A_wo: jax.Array,
    B_x: jax.Array,
    B_w_r: jax.Array,
    B_w_gate: jax.Array,
    B_w_up: jax.Array,
    B_w_down: jax.Array,
):
    del B_x
    bf16, f32 = jnp.bfloat16, jnp.float32
    x2 = A_x.reshape(1, D)
    kt = jnp.swapaxes(A_k_cache, 2, 3).reshape(H, DH, SK)
    vt = jnp.swapaxes(A_v_cache, 2, 3).reshape(H, DH, SK)
    wq3 = A_wq.reshape(WQ_G, WQ_R, H * DH)
    wo3 = A_wo.reshape(WO_G, WO_R, D)
    hbm = pl.BlockSpec(memory_space=pl.ANY)
    dma = pltpu.SemaphoreType.DMA
    out = pl.pallas_call(
        _kernel,
        in_specs=[hbm] * 9,
        out_specs=pl.BlockSpec(memory_space=pltpu.VMEM),
        out_shape=jax.ShapeDtypeStruct((1, D), A_x.dtype),
        scratch_shapes=[
            pltpu.VMEM((RK, DH, W), bf16),
            pltpu.VMEM((RV, DH, W), bf16),
            pltpu.VMEM((WQ_G, WQ_R, H * DH), bf16),
            pltpu.VMEM((WO_G, WO_R, D), bf16),
            pltpu.VMEM((D, F), bf16),
            pltpu.VMEM((D, F), bf16),
            pltpu.VMEM((F, D), bf16),
            pltpu.VMEM((1, D), bf16),
            pltpu.VMEM((D,), bf16),
            pltpu.VMEM((8, D), bf16),
            pltpu.VMEM((H, DH), f32),
            pltpu.VMEM((NC, CH), f32),
            pltpu.VMEM((H, DH), f32),
            pltpu.VMEM((8, D), f32),
            dma((RK,)),
            dma((RV,)),
            dma((2,)),
            dma((H // 2,)),
            dma((1,)),
            dma((2 * (D // GB),)),
            dma((2 * (F // DN_BLK),)),
        ],
        compiler_params=pltpu.CompilerParams(
            vmem_limit_bytes=64 * 1024 * 1024,
            disable_bounds_checks=True,
            disable_semaphore_checks=True,
        ),
    )(x2, kt, vt, wq3, wo3, B_w_r, B_w_gate, B_w_up, B_w_down)
    return out.reshape(1, 1, D)
```
